```python
import jax
import jax.numpy as jnp

def _softmax(x, axis=-1):
    return jax.nn.softmax(x, axis=axis)
def _gelu(x):
    return jax.nn.gelu(x, approximate=True)
def _silu(x):
    return jax.nn.silu(x)
def _sigmoid(x):
    return jax.nn.sigmoid(x)
def _layernorm(x, axis=-1, eps=1e-5):
    m = jnp.mean(x, axis=axis, keepdims=True)
    v = jnp.var(x, axis=axis, keepdims=True)
    return (x - m) / jnp.sqrt(v + eps)
def _scatter_add(tgt, idx, src, axis=0):
    return tgt.at[idx].add(src)
def _segment_sum(src, seg, n):
    return jax.ops.segment_sum(src, seg, n)
class _Rng:
    def __init__(self, key):
        self._k = key
    def _next(self):
        self._k, sub = jax.random.split(self._k)
        return sub
    def normal(self, shape):
        return jax.random.normal(self._next(), shape, dtype=jnp.bfloat16)
    def randint(self, lo, hi, shape):
        return jax.random.randint(self._next(), shape, lo, hi, dtype=jnp.int32)
    def uniform(self, shape, lo=0.0, hi=1.0):
        return jax.random.uniform(self._next(), shape, jnp.bfloat16, lo, hi)
    def permutation(self, n):
        return jax.random.permutation(self._next(), n)


kernel_name = 'interleave_layers__softmax_full_mha__ssm_conv_h3__prompt'

def setup_inputs():
    _rng = _Rng(jax.random.key(int.from_bytes(__import__("os").urandom(4), "little")))
    _w = (lambda a: (lambda t: t.astype(jnp.bfloat16) if jnp.issubdtype(t.dtype, jnp.floating) else t)(jnp.asarray(a)))
    def _A_setup():
        B, S, D = 1, 2048, 1024
        return {
            "x": _w((lambda *s: _rng.normal(s) * 0.05)(B, S, D)),
            "wqkv": _w((lambda *s: _rng.normal(s) * 0.05)(D, 3 * D)),
            "wo": _w((lambda *s: _rng.normal(s) * 0.05)(D, D)),
        }
    _A_in = _A_setup()

    def _B_setup():
        B, S, D = 1, 2048, 1024
        ks = 4
        return {
            "q": _w((lambda *s: _rng.normal(s) * 0.05)(B, S, D)),
            "k": _w((lambda *s: _rng.normal(s) * 0.05)(B, S, D)),
            "v": _w((lambda *s: _rng.normal(s) * 0.05)(B, S, D)),
            "shift_k": _w((lambda *s: _rng.normal(s) * 0.05)(D, ks) * 0.5),
            "ssm_k": _w((lambda *s: _rng.normal(s) * 0.05)(D, S) * (1.0 / S ** 0.5)),
            "ssm_D": _w((lambda *s: _rng.normal(s) * 0.05)(D)),
        }
    _B_in = _B_setup()

    return {
        "A_x": _A_in["x"],
        "A_wqkv": _A_in["wqkv"],
        "A_wo": _A_in["wo"],
        "B_q": _B_in["q"],
        "B_k": _B_in["k"],
        "B_v": _B_in["v"],
        "B_shift_k": _B_in["shift_k"],
        "B_ssm_k": _B_in["ssm_k"],
        "B_ssm_D": _B_in["ssm_D"],
    }

def reference(A_x, A_wqkv, A_wo, B_q, B_k, B_v, B_shift_k, B_ssm_k, B_ssm_D):
    def _A_ref(x, wqkv, wo):
        B, S, D = x.shape
        H = 32; Dh = D // H
        qkv = (lambda x, *d: x.transpose(*d))((x @ wqkv).reshape(B, S, 3, H, Dh), 2, 0, 3, 1, 4)
        q, k, v = qkv[0], qkv[1], qkv[2]
        scale = Dh ** -0.5
        scores = jnp.einsum("bhqd,bhkd->bhqk", q, k) * scale
        p = _softmax(scores, axis=-1)
        o = jnp.einsum("bhqk,bhkd->bhqd", p, v)
        return (lambda x, *d: x.transpose(*d))(o, 0, 2, 1, 3).reshape(B, S, D) @ wo

    def _B_ref(q, k, v, shift_k, ssm_k, ssm_D):
        B, S, D = q.shape
        ks = shift_k.shape[-1]
        k_pad = jnp.pad(k, ((0, 0), (ks - 1, 0), (0, 0)))
        k_shift = jnp.zeros_like(k)
        for t in range(ks):
            k_shift = k_shift + k_pad[:, t:t + S, :] * shift_k[:, ks - 1 - t][None, None, :]
        kv = k_shift * v
        L = 2 * S
        kv_pad = jnp.pad(kv, ((0, 0), (0, S), (0, 0)))
        kf_pad = jnp.pad(ssm_k, ((0, 0), (0, S)))
        kv_f = (lambda x, axes=(-2,-1): jnp.fft.rfft2(x.astype(jnp.float32), axes=axes))(kv_pad[:, None, :, :], axes=(1, 2))
        kf_f = (lambda x, axes=(-2,-1): jnp.fft.rfft2(x.astype(jnp.float32), axes=axes))(kf_pad[:, None, :], axes=(1, 2))
        kf_f = (lambda x, *d: x.transpose(*d))(kf_f, 1, 2, 0)
        y_f = kv_f * kf_f[None, :, :, :]
        y = (lambda x, s, axes=(-2,-1): jnp.fft.irfft2(x, s=s, axes=axes).astype(jnp.bfloat16))(y_f, (1, L), axes=(1, 2))[:, 0, :S, :]
        y = y + kv * ssm_D[None, None, :]
        return q * y

    x = A_x
    x = x + _A_ref(_layernorm(x, axis=-1), A_wqkv, A_wo)
    x = x + _B_ref(_layernorm(x, axis=-1), B_k, B_v, B_shift_k, B_ssm_k, B_ssm_D)
    x = x + _A_ref(_layernorm(x, axis=-1), A_wqkv, A_wo)
    x = x + _B_ref(_layernorm(x, axis=-1), B_k, B_v, B_shift_k, B_ssm_k, B_ssm_D)
    return x
```

```python
import functools

import jax
import jax.numpy as jnp
import numpy as np
from jax import lax
import jax.experimental.pallas as pl
import jax.experimental.pallas.tpu as pltpu

S, D, H, DH = 2048, 1024, 32, 32
VR = 48
TQ = 512
KC = 512
RC = 512
L = 128
NB = S // L
NT = (((1,), (1,)), ((), ()))
TN = (((0,), (0,)), ((), ()))
F32, BF16 = jnp.float32, jnp.bfloat16

_th = np.pi * np.outer(np.arange(L) + 0.5, np.arange(L)) / L
_FWD = np.concatenate([np.cos(_th), -np.sin(_th)], 0)
_INV = np.concatenate([np.cos(_th).T, -np.sin(_th).T], 1) / L
_EYE = np.eye(16, 4)


def _ln(x):
    m = jnp.mean(x, axis=-1, keepdims=True)
    c = x - m
    v = jnp.mean(c * c, axis=-1, keepdims=True)
    return c * lax.rsqrt(v + 1e-5)


def _kernel(x_hbm, wqkv_hbm, wo_hbm, k_hbm, v_hbm, ssmk_hbm, shift_ref, ssmd_ref,
            fwd_ref, inv_ref, eye_ref, out_hbm,
            xin, x_scr, wqkv, wo, wvt, q_scr, k_scr, vt_scr, ot_scr, s_scr, m_scr,
            bk, bv, bh, y_scr, kvf, hf, yf, sems, osems):
    nchunk = S // RC
    in_copies = [
        pltpu.make_async_copy(x_hbm, xin, sems.at[0]),
        pltpu.make_async_copy(wqkv_hbm, wqkv, sems.at[1]),
        pltpu.make_async_copy(wo_hbm, wo, sems.at[2]),
        pltpu.make_async_copy(k_hbm, bk, sems.at[3]),
        pltpu.make_async_copy(v_hbm, bv, sems.at[4]),
        pltpu.make_async_copy(ssmk_hbm, bh, sems.at[5]),
    ]
    for c in in_copies:
        c.start()

    row = lax.broadcasted_iota(jnp.int32, (H, VR - DH, S), 1)
    vt_scr[:, DH:VR, :] = jnp.where(row == 0, 1.0, 0.0).astype(BF16)

    def proj(r0, x):
        h = _ln(x).astype(BF16)
        rows = pl.ds(r0, RC)
        qs = DH ** -0.5 * np.log2(np.e)
        for g in range(D // 128):
            qk = jnp.dot(h, wqkv[:, g * 128:(g + 1) * 128], preferred_element_type=F32)
            q_scr[g, rows, :] = (qk * qs).astype(BF16)
        for g in range(D // 128):
            qk = jnp.dot(h, wqkv[:, D + g * 128:D + (g + 1) * 128], preferred_element_type=F32)
            k_scr[g, rows, :] = qk.astype(BF16)
        vt = lax.dot_general(wvt[...], h, NT, preferred_element_type=F32)
        vt_scr[:, 0:DH, rows] = vt.astype(BF16).reshape(H, DH, RC)

    def attention():
        nq = S // TQ
        ni = H * nq
        lane = lax.broadcasted_iota(jnp.int32, (TQ, 128), 1) // DH

        def stage_a(n, slot):
            h, qi = n // nq, n % nq
            g = h // 4
            q = q_scr[g, pl.ds(pl.multiple_of(qi * TQ, TQ), TQ), :]
            qm = jnp.where(lane == h % 4, q, jnp.zeros_like(q))
            m = None
            for c in range(S // KC):
                s = lax.dot_general(k_scr[g, c * KC:(c + 1) * KC, :], qm, NT,
                                    preferred_element_type=F32)
                s_scr[slot, c * KC:(c + 1) * KC, :] = s
                mc = jnp.max(s.reshape(KC // 8, 8, TQ), axis=0)
                m = mc if m is None else jnp.maximum(m, mc)
            m_scr[slot] = jnp.broadcast_to(jnp.max(m, axis=0, keepdims=True), (8, TQ))

        def stage_b(n, slot):
            h, qi = n // nq, n % nq
            m = m_scr[slot][0:1, :]
            o = None
            for c in range(S // KC):
                p = jnp.exp2(s_scr[slot, c * KC:(c + 1) * KC, :] - m).astype(BF16)
                oc = jnp.dot(vt_scr[h, :, c * KC:(c + 1) * KC], p, preferred_element_type=F32)
                o = oc if o is None else o + oc
            ot_scr[pl.ds(pl.multiple_of(h * DH, DH), DH), pl.ds(pl.multiple_of(qi * TQ, TQ), TQ)] = (
                o[0:DH] * (1.0 / o[DH:DH + 1])).astype(BF16)

        stage_a(0, 0)

        def body(i, c):
            n = 2 * i + 1
            stage_a(n, 1)
            stage_b(n - 1, 0)
            stage_a(n + 1, 0)
            stage_b(n, 1)
            return c

        lax.fori_loop(0, ni // 2 - 1, body, 0)
        stage_a(ni - 1, 1)
        stage_b(ni - 2, 0)
        stage_b(ni - 1, 1)

    def conv():
        taps = lax.dot_general(eye_ref[...], shift_ref[...], NT, preferred_element_type=F32)
        ssmd = ssmd_ref[...].astype(F32)
        fwd = fwd_ref[...]
        sgn = 1.0 - 2.0 * (lax.broadcasted_iota(jnp.int32, (L, D), 0) % 2).astype(F32)

        def fwd_block(j, prev):
            r0 = pl.multiple_of(j * L, L)
            cur = bk[pl.ds(r0, L), :].astype(F32)
            p0 = pl.multiple_of(jnp.maximum(r0 - 16, 0), 16)
            hist = jnp.where(j > 0, bk[pl.ds(p0, 16), :].astype(F32), 0.0)
            ext = jnp.concatenate([hist, cur], axis=0)
            ks = cur * taps[0:1]
            for d in range(1, 4):
                ks = ks + pltpu.roll(ext, d, 0)[16:] * taps[d:d + 1]
            kv = (ks * bv[pl.ds(r0, L), :].astype(F32))
            y_scr[pl.ds(r0, L), :] = kv * ssmd
            kvf[j] = jnp.dot(fwd, kv.astype(BF16), preferred_element_type=F32)
            g = lax.dot_general(fwd, bh[:, pl.ds(r0, L)], NT, preferred_element_type=F32)
            gr, gi = g[:L], g[L:]
            pr, pi = prev
            hf[j, 0:L] = gr - sgn * pi
            hf[j, L:] = gi + sgn * pr
            return gr, gi

        z = jnp.zeros((L, D), F32)
        lax.fori_loop(0, NB, fwd_block, (z, z))

        def mix(t, c):
            re = pl.ds(pl.multiple_of(t * 8, 8), 8)
            im = pl.ds(pl.multiple_of(L + t * 8, 8), 8)
            for i in range(NB):
                ar = ai = None
                for j in range(i + 1):
                    kr, ki = kvf[j, re, :], kvf[j, im, :]
                    hr, hi = hf[i - j, re, :], hf[i - j, im, :]
                    tr, ti = kr * hr - ki * hi, kr * hi + ki * hr
                    ar = tr if ar is None else ar + tr
                    ai = ti if ai is None else ai + ti
                yf[i, re, :] = ar
                yf[i, im, :] = ai
            return c

        lax.fori_loop(0, L // 8, mix, 0)

        def inv_block(i, c):
            rows = pl.ds(pl.multiple_of(i * L, L), L)
            y_scr[rows, :] += jnp.dot(inv_ref[...], yf[i].astype(BF16), preferred_element_type=F32)
            return c

        lax.fori_loop(0, NB, inv_block, 0)

    def out_copy(c):
        rows = pl.ds(c * RC, RC)
        return pltpu.make_async_copy(xin.at[rows], out_hbm.at[rows], osems.at[c])

    def post(last):
        def body(c, carry):
            r0 = pl.multiple_of(c * RC, RC)
            rows = pl.ds(r0, RC)
            x = x_scr[rows, :] + lax.dot_general(ot_scr[:, rows], wo[...], TN,
                                                 preferred_element_type=F32)
            x = x + _ln(x) * y_scr[rows, :]
            if last:
                xin[rows, :] = x.astype(BF16)
                out_copy(c).start()
            else:
                x_scr[rows, :] = x
                proj(r0, x)
            return carry
        lax.fori_loop(0, nchunk, body, 0)

    in_copies[0].wait()
    in_copies[1].wait()
    wvt[...] = wqkv[:, 2 * D:].astype(F32).T.astype(BF16)

    def first(c, carry):
        r0 = pl.multiple_of(c * RC, RC)
        x = xin[pl.ds(r0, RC), :].astype(F32)
        x_scr[pl.ds(r0, RC), :] = x
        proj(r0, x)
        return carry

    lax.fori_loop(0, nchunk, first, 0)
    attention()
    for c in in_copies[2:]:
        c.wait()
    conv()
    post(False)
    attention()
    post(True)
    for c in range(nchunk):
        out_copy(c).wait()


@jax.jit
def pallas_interleave_layers__softmax_full_mha__ssm_conv_h3__prompt_kernel(
    A_x: jax.Array,
    A_wqkv: jax.Array,
    A_wo: jax.Array,
    B_q: jax.Array,
    B_k: jax.Array,
    B_v: jax.Array,
    B_shift_k: jax.Array,
    B_ssm_k: jax.Array,
    B_ssm_D: jax.Array,
):
    del B_q
    hbm = pl.BlockSpec(memory_space=pl.ANY)
    vmem = pl.BlockSpec(memory_space=pltpu.VMEM)
    out = pl.pallas_call(
        _kernel,
        in_specs=[hbm] * 6 + [vmem] * 5,
        out_specs=hbm,
        out_shape=jax.ShapeDtypeStruct((S, D), BF16),
        scratch_shapes=[
            pltpu.VMEM((S, D), BF16),
            pltpu.VMEM((S, D), F32),
            pltpu.VMEM((D, 3 * D), BF16),
            pltpu.VMEM((D, D), BF16),
            pltpu.VMEM((D, D), BF16),
            pltpu.VMEM((D // 128, S, 128), BF16),
            pltpu.VMEM((D // 128, S, 128), BF16),
            pltpu.VMEM((H, VR, S), BF16),
            pltpu.VMEM((D, S), BF16),
            pltpu.VMEM((2, S, TQ), F32),
            pltpu.VMEM((2, 8, TQ), F32),
            pltpu.VMEM((S, D), BF16),
            pltpu.VMEM((S, D), BF16),
            pltpu.VMEM((D, S), BF16),
            pltpu.VMEM((S, D), F32),
            pltpu.VMEM((NB, 2 * L, D), F32),
            pltpu.VMEM((NB, 2 * L, D), F32),
            pltpu.VMEM((NB, 2 * L, D), F32),
            pltpu.SemaphoreType.DMA((6,)),
            pltpu.SemaphoreType.DMA((S // RC,)),
        ],
        compiler_params=pltpu.CompilerParams(vmem_limit_bytes=127 * 2 ** 20),
    )(A_x.reshape(S, D), A_wqkv, A_wo, B_k.reshape(S, D), B_v.reshape(S, D), B_ssm_k,
      B_shift_k, B_ssm_D.reshape(1, D),
      _FWD.astype(BF16), _INV.astype(BF16), _EYE.astype(BF16))
    return out.reshape(1, S, D)
```

```python
import functools

import jax
import jax.numpy as jnp
import numpy as np
from jax import lax
import jax.experimental.pallas as pl
import jax.experimental.pallas.tpu as pltpu

S, D, H, DH = 2048, 1024, 32, 32
VR = 48
TQ = 512
KC = 512
RC = 256
L = 128
NB = S // L
NT = (((1,), (1,)), ((), ()))
TN = (((0,), (0,)), ((), ()))
F32, BF16 = jnp.float32, jnp.bfloat16

_th = np.pi * np.outer(np.arange(L) + 0.5, np.arange(L)) / L
_FWD = np.concatenate([np.cos(_th), -np.sin(_th)], 0)
_INV = np.concatenate([np.cos(_th).T, -np.sin(_th).T], 1) / L
_EYE = np.eye(16, 4)


def _ln(x):
    m = jnp.mean(x, axis=-1, keepdims=True)
    c = x - m
    v = jnp.mean(c * c, axis=-1, keepdims=True)
    return c * lax.rsqrt(v + 1e-5)


def _kernel(x_hbm, wqkv_hbm, wo_hbm, k_hbm, v_hbm, ssmk_hbm, shift_ref, ssmd_ref,
            fwd_ref, inv_ref, eye_ref, out_hbm,
            xin, x_scr, wqkv, wo, wvt, q_scr, k_scr, vt_scr, ot_scr, s_scr, m_scr,
            bk, bv, bh, y_scr, kvf, hf, yf, sems, osems):
    nchunk = S // RC
    in_copies = [
        pltpu.make_async_copy(x_hbm, xin, sems.at[0]),
        pltpu.make_async_copy(wqkv_hbm, wqkv, sems.at[1]),
        pltpu.make_async_copy(wo_hbm, wo, sems.at[2]),
        pltpu.make_async_copy(k_hbm, bk, sems.at[3]),
        pltpu.make_async_copy(v_hbm, bv, sems.at[4]),
        pltpu.make_async_copy(ssmk_hbm, bh, sems.at[5]),
    ]
    for c in in_copies[:2]:
        c.start()

    row = lax.broadcasted_iota(jnp.int32, (H, VR - DH, S), 1)
    vt_scr[:, DH:VR, :] = jnp.where(row == 0, 1.0, 0.0).astype(BF16)

    def proj(r0, x):
        h = _ln(x).astype(BF16)
        rows = pl.ds(r0, RC)
        qs = DH ** -0.5 * np.log2(np.e)
        qk = jnp.dot(h, wqkv[:, :2 * D], preferred_element_type=F32)
        for g in range(D // 128):
            q_scr[g, rows, :] = (qk[:, g * 128:(g + 1) * 128] * qs).astype(BF16)
            k_scr[g, rows, :] = qk[:, D + g * 128:D + (g + 1) * 128].astype(BF16)
        vt = lax.dot_general(wvt[...], h, NT, preferred_element_type=F32)
        vt_scr[:, 0:DH, rows] = vt.astype(BF16).reshape(H, DH, RC)

    def attention(filler=None):
        nq = S // TQ
        ni = H * nq
        lane = lax.broadcasted_iota(jnp.int32, (TQ, 128), 1) // DH

        def stage_a(n, slot):
            h, qi = n // nq, n % nq
            g = h // 4
            q = q_scr[g, pl.ds(pl.multiple_of(qi * TQ, TQ), TQ), :]
            qm = jnp.where(lane == h % 4, q, jnp.zeros_like(q))
            m = None
            for c in range(S // KC):
                s = lax.dot_general(k_scr[g, c * KC:(c + 1) * KC, :], qm, NT,
                                    preferred_element_type=F32)
                s_scr[slot, c * KC:(c + 1) * KC, :] = s
                mc = jnp.max(s.reshape(KC // 8, 8, TQ), axis=0)
                m = mc if m is None else jnp.maximum(m, mc)
            m_scr[slot] = jnp.broadcast_to(jnp.max(m, axis=0, keepdims=True), (8, TQ))

        def stage_b(n, slot):
            h, qi = n // nq, n % nq
            m = m_scr[slot][0:1, :]
            o = None
            for c in range(S // KC):
                p = jnp.exp2(s_scr[slot, c * KC:(c + 1) * KC, :] - m).astype(BF16)
                oc = jnp.dot(vt_scr[h, :, c * KC:(c + 1) * KC], p, preferred_element_type=F32)
                o = oc if o is None else o + oc
            ot_scr[pl.ds(pl.multiple_of(h * DH, DH), DH), pl.ds(pl.multiple_of(qi * TQ, TQ), TQ)] = (
                o[0:DH] * (1.0 / o[DH:DH + 1])).astype(BF16)

        stage_a(0, 0)

        def body(i, c):
            n = 2 * i + 1
            fill = filler if filler is not None else (lambda *a: None)
            stage_a(n, 1)
            stage_b(n - 1, 0)
            stage_a(n + 1, 0)
            stage_b(n, 1)
            for c2 in range(8):
                fill(i, c2)
            return c

        lax.fori_loop(0, ni // 2 - 1, body, 0)
        stage_a(ni - 1, 1)
        stage_b(ni - 2, 0)
        stage_b(ni - 1, 1)
        if filler is not None:
            for c in range(8):
                filler(ni // 2 - 1, c)

    def conv_fwd():
        taps = lax.dot_general(eye_ref[...], shift_ref[...], NT, preferred_element_type=F32)
        ssmd = ssmd_ref[...].astype(F32)
        fwd = fwd_ref[...]
        sgn = 1.0 - 2.0 * (lax.broadcasted_iota(jnp.int32, (L, D), 0) % 2).astype(F32)

        def fwd_block(j, prev):
            r0 = pl.multiple_of(j * L, L)
            cur = bk[pl.ds(r0, L), :].astype(F32)
            p0 = pl.multiple_of(jnp.maximum(r0 - 16, 0), 16)
            hist = jnp.where(j > 0, bk[pl.ds(p0, 16), :].astype(F32), 0.0)
            ext = jnp.concatenate([hist, cur], axis=0)
            ks = cur * taps[0:1]
            for d in range(1, 4):
                ks = ks + pltpu.roll(ext, d, 0)[16:] * taps[d:d + 1]
            kv = (ks * bv[pl.ds(r0, L), :].astype(F32))
            y_scr[pl.ds(r0, L), :] = kv * ssmd
            kvf[j] = jnp.dot(fwd, kv.astype(BF16), preferred_element_type=F32)
            g = lax.dot_general(fwd, bh[:, pl.ds(r0, L)], NT, preferred_element_type=F32)
            gr, gi = g[:L], g[L:]
            pr, pi = prev
            hf[j, 0:L] = gr - sgn * pi
            hf[j, L:] = gi + sgn * pr
            return gr, gi

        z = jnp.zeros((L, D), F32)
        lax.fori_loop(0, NB, fwd_block, (z, z), unroll=2)

    def conv_mix(t, part):
        re = pl.ds(pl.multiple_of((t // 4) * 8, 8), 8)
        im = pl.ds(pl.multiple_of(L + (t // 4) * 8, 8), 8)
        ch = pl.ds(pl.multiple_of((t % 4) * 256, 256), 256)
        for i in (part, NB - 1 - part):
            ar = ai = None
            for j in range(i + 1):
                kr, ki = kvf[j, re, ch], kvf[j, im, ch]
                hr, hi = hf[i - j, re, ch], hf[i - j, im, ch]
                tr, ti = kr * hr - ki * hi, kr * hi + ki * hr
                ar = tr if ar is None else ar + tr
                ai = ti if ai is None else ai + ti
            yf[i, re, ch] = ar
            yf[i, im, ch] = ai

    def conv_inv():
        def inv_block(i, c):
            rows = pl.ds(pl.multiple_of(i * L, L), L)
            y_scr[rows, :] += jnp.dot(inv_ref[...], yf[i].astype(BF16), preferred_element_type=F32)
            return c

        lax.fori_loop(0, NB, inv_block, 0)

    def out_copy(c):
        rows = pl.ds(c * RC, RC)
        return pltpu.make_async_copy(xin.at[rows], out_hbm.at[rows], osems.at[c])

    def post(last):
        def body(c, carry):
            r0 = pl.multiple_of(c * RC, RC)
            rows = pl.ds(r0, RC)
            x = x_scr[rows, :] + lax.dot_general(ot_scr[:, rows], wo[...], TN,
                                                 preferred_element_type=F32)
            x = x + _ln(x) * y_scr[rows, :]
            if last:
                xin[rows, :] = x.astype(BF16)
                out_copy(c).start()
            else:
                x_scr[rows, :] = x
                proj(r0, x)
            return carry
        lax.fori_loop(0, nchunk, body, 0)

    in_copies[0].wait()
    in_copies[1].wait()
    for c in in_copies[2:]:
        c.start()
    wvt[...] = wqkv[:, 2 * D:].astype(F32).T.astype(BF16)

    def first(c, carry):
        r0 = pl.multiple_of(c * RC, RC)
        x = xin[pl.ds(r0, RC), :].astype(F32)
        x_scr[pl.ds(r0, RC), :] = x
        proj(r0, x)
        return carry

    lax.fori_loop(0, nchunk, first, 0)
    for c in in_copies[2:]:
        c.wait()
    conv_fwd()
    attention(conv_mix)
    conv_inv()
    post(False)
    attention()
    post(True)
    for c in range(nchunk):
        out_copy(c).wait()


@jax.jit
def pallas_interleave_layers__softmax_full_mha__ssm_conv_h3__prompt_kernel(
    A_x: jax.Array,
    A_wqkv: jax.Array,
    A_wo: jax.Array,
    B_q: jax.Array,
    B_k: jax.Array,
    B_v: jax.Array,
    B_shift_k: jax.Array,
    B_ssm_k: jax.Array,
    B_ssm_D: jax.Array,
):
    del B_q
    hbm = pl.BlockSpec(memory_space=pl.ANY)
    vmem = pl.BlockSpec(memory_space=pltpu.VMEM)
    out = pl.pallas_call(
        _kernel,
        in_specs=[hbm] * 6 + [vmem] * 5,
        out_specs=hbm,
        out_shape=jax.ShapeDtypeStruct((S, D), BF16),
        scratch_shapes=[
            pltpu.VMEM((S, D), BF16),
            pltpu.VMEM((S, D), F32),
            pltpu.VMEM((D, 3 * D), BF16),
            pltpu.VMEM((D, D), BF16),
            pltpu.VMEM((D, D), BF16),
            pltpu.VMEM((D // 128, S, 128), BF16),
            pltpu.VMEM((D // 128, S, 128), BF16),
            pltpu.VMEM((H, VR, S), BF16),
            pltpu.VMEM((D, S), BF16),
            pltpu.VMEM((2, S, TQ), F32),
            pltpu.VMEM((2, 8, TQ), F32),
            pltpu.VMEM((S, D), BF16),
            pltpu.VMEM((S, D), BF16),
            pltpu.VMEM((D, S), BF16),
            pltpu.VMEM((S, D), F32),
            pltpu.VMEM((NB, 2 * L, D), F32),
            pltpu.VMEM((NB, 2 * L, D), F32),
            pltpu.VMEM((NB, 2 * L, D), F32),
            pltpu.SemaphoreType.DMA((6,)),
            pltpu.SemaphoreType.DMA((S // RC,)),
        ],
        compiler_params=pltpu.CompilerParams(vmem_limit_bytes=127 * 2 ** 20),
    )(A_x.reshape(S, D), A_wqkv, A_wo, B_k.reshape(S, D), B_v.reshape(S, D), B_ssm_k,
      B_shift_k, B_ssm_D.reshape(1, D),
      _FWD.astype(BF16), _INV.astype(BF16), _EYE.astype(BF16))
    return out.reshape(1, S, D)
```
